```python
import jax
import jax.numpy as jnp

def _softmax(x, axis=-1):
    return jax.nn.softmax(x, axis=axis)
def _gelu(x):
    return jax.nn.gelu(x, approximate=True)
def _silu(x):
    return jax.nn.silu(x)
def _sigmoid(x):
    return jax.nn.sigmoid(x)
def _layernorm(x, axis=-1, eps=1e-5):
    m = jnp.mean(x, axis=axis, keepdims=True)
    v = jnp.var(x, axis=axis, keepdims=True)
    return (x - m) / jnp.sqrt(v + eps)
def _scatter_add(tgt, idx, src, axis=0):
    return tgt.at[idx].add(src)
def _segment_sum(src, seg, n):
    return jax.ops.segment_sum(src, seg, n)
class _Rng:
    def __init__(self, key):
        self._k = key
    def _next(self):
        self._k, sub = jax.random.split(self._k)
        return sub
    def normal(self, shape):
        return jax.random.normal(self._next(), shape, dtype=jnp.bfloat16)
    def randint(self, lo, hi, shape):
        return jax.random.randint(self._next(), shape, lo, hi, dtype=jnp.int32)
    def uniform(self, shape, lo=0.0, hi=1.0):
        return jax.random.uniform(self._next(), shape, jnp.bfloat16, lo, hi)
    def permutation(self, n):
        return jax.random.permutation(self._next(), n)


kernel_name = 'parallel_sum__sliding_local_dilated__mixer_token_mlp__prompt'

def setup_inputs():
    _rng = _Rng(jax.random.key(int.from_bytes(__import__("os").urandom(4), "little")))
    _w = (lambda a: (lambda t: t.astype(jnp.bfloat16) if jnp.issubdtype(t.dtype, jnp.floating) else t)(jnp.asarray(a)))
    def _A_setup():
        B, S, D = 1, 2048, 448
        return {
            "x": _w((lambda *s: _rng.normal(s) * 0.05)(B, S, D)),
            "wqkv": _w((lambda *s: _rng.normal(s) * 0.05)(D, 3 * D)),
            "wo": _w((lambda *s: _rng.normal(s) * 0.05)(D, D)),
        }
    _A_in = _A_setup()

    def _B_setup():
        B, S, D, F = 1, 2048, 448, 1792
        return {
            "x": _w((lambda *s: _rng.normal(s) * 0.05)(B, S, D)),
            "w1": _w((lambda *s: _rng.normal(s) * 0.05)(S, F) * (S ** -0.5)),
            "b1": _w((lambda *s: _rng.normal(s) * 0.05)(F) * 0.02),
            "w2": _w((lambda *s: _rng.normal(s) * 0.05)(F, S) * (F ** -0.5)),
            "b2": _w((lambda *s: _rng.normal(s) * 0.05)(S) * 0.02),
        }
    _B_in = _B_setup()

    return {
        "A_x": _A_in["x"],
        "A_wqkv": _A_in["wqkv"],
        "A_wo": _A_in["wo"],
        "B_x": _B_in["x"],
        "B_w1": _B_in["w1"],
        "B_b1": _B_in["b1"],
        "B_w2": _B_in["w2"],
        "B_b2": _B_in["b2"],
    }

def reference(A_x, A_wqkv, A_wo, B_x, B_w1, B_b1, B_w2, B_b2):
    def _A_ref(x, wqkv, wo):
        B, S, D = x.shape
        H = 16; Dh = D // H
        W, dil = 8, 2
        qkv = (lambda x, *d: x.transpose(*d))((x @ wqkv).reshape(B, S, 3, H, Dh), 2, 0, 3, 1, 4)
        q, k, v = qkv[0], qkv[1], qkv[2]
        scale = Dh ** -0.5
        pos = jnp.arange(S)
        off = jnp.arange(W) * dil
        idx = pos[:, None] - off[None, :]
        mask = idx >= 0
        idx_c = jnp.where(mask, idx, 0).reshape(-1)
        kg = k[:, :, idx_c, :].reshape(B, H, S, W, Dh)
        vg = v[:, :, idx_c, :].reshape(B, H, S, W, Dh)
        logits = jnp.einsum("bhsd,bhswd->bhsw", q, kg) * scale
        logits = jnp.where(mask[None, None, :, :], logits, -1e9)
        attn = _softmax(logits, axis=-1)
        o = jnp.einsum("bhsw,bhswd->bhsd", attn, vg)
        return (lambda x, *d: x.transpose(*d))(o, 0, 2, 1, 3).reshape(B, S, D) @ wo

    def _B_ref(x, w1, b1, w2, b2):
        B, S, D = x.shape
        h = _layernorm(x, axis=-1)
        u = jnp.einsum("bsd,sf->bdf", h, w1) + b1
        u = _gelu(u)
        y = jnp.einsum("bdf,fs->bds", u, w2) + b2
        return (lambda x, *d: x.transpose(*d))(y, 0, 2, 1)

    x = A_x
    xn = _layernorm(x, axis=-1)
    return x + _A_ref(xn, A_wqkv, A_wo) + _B_ref(xn, B_w1, B_b1, B_w2, B_b2)
```

```python
import jax
import jax.numpy as jnp
import jax.experimental.pallas as pl
import jax.experimental.pallas.tpu as pltpu

S, D, F, H, Dh, W = 2048, 448, 1792, 16, 28, 8
CH = 512
PAD = 128
f32, bf16 = jnp.float32, jnp.bfloat16


def _kernel(x_ref, wqkv_ref, wo_ref, w1_hbm, b1_ref, w2_hbm, b2_ref, o_ref,
            w1_v, w2_v, sems, xnT, wT, ws, wos, qs, ks, vs, os_, us, woT, ov):
    x_ref = x_ref.at[0]
    o_ref = o_ref.at[0]
    nF = F // 256
    c1 = [pltpu.make_async_copy(w1_hbm.at[:, pl.ds(i * 256, 256)], w1_v.at[:, pl.ds(i * 256, 256)], sems.at[0, i])
          for i in range(nF)]
    c2 = [pltpu.make_async_copy(w2_hbm.at[pl.ds(i * 256, 256), :], w2_v.at[pl.ds(i * 256, 256), :], sems.at[1, i])
          for i in range(nF)]
    for c in c1 + c2:
        c.start()

    wf = wqkv_ref[...].astype(f32)
    wp = jnp.concatenate([wf, jnp.zeros((D, 64), f32)], axis=1)
    wp = jnp.concatenate([wp, jnp.zeros((64, 1408), f32)], axis=0)
    wt = wp.T[:3 * D, :]
    for j in range(4):
        wT[j] = wt[:, j * 128:(j + 1) * 128]

    def gather(r0):
        return jnp.concatenate([wT[j, pl.ds(r0, H, stride=Dh), :] for j in range(4)], axis=1)[:, :D]
    scale = Dh ** -0.5
    for part in range(3):
        for d in range(Dh):
            blk = gather(part * D + d)
            if part == 0:
                blk = blk * scale
            ws[pl.ds(part * D + d * H, H), :] = blk.astype(bf16)
    wof = jnp.concatenate([wo_ref[...].astype(f32), jnp.zeros((D, 64), f32)], axis=1)
    for j in range(4):
        wT[j, pl.ds(0, D), :] = wof[:, j * 128:(j + 1) * 128]
    for d in range(Dh):
        wos[pl.ds(d * H, H), :] = gather(d).astype(bf16)

    wq = jnp.concatenate([wos[...].astype(f32), jnp.zeros((D, 64), f32)], axis=1)
    wq = jnp.concatenate([wq, jnp.zeros((64, 512), f32)], axis=0)
    woT[...] = wq.T[:D, :D].astype(bf16)
    for c in range(S // CH):
        xf = x_ref[:, pl.ds(c * CH, CH)].astype(f32)
        m = jnp.mean(xf, axis=0, keepdims=True)
        xc = xf - m
        v = jnp.mean(xc * xc, axis=0, keepdims=True)
        xnT[:, pl.ds(c * CH, CH)] = (xc / jnp.sqrt(v + 1e-5)).astype(bf16)

    ks[:, pl.ds(0, PAD)] = jnp.zeros((D, PAD), f32)
    vs[:, pl.ds(0, PAD)] = jnp.zeros((D, PAD), f32)
    for c in range(S // CH):
        xc = xnT[:, pl.ds(c * CH, CH)]
        qs[:, pl.ds(c * CH, CH)] = jnp.dot(ws[pl.ds(0, D), :], xc, preferred_element_type=f32)
        ks[:, pl.ds(PAD + c * CH, CH)] = jnp.dot(ws[pl.ds(D, D), :], xc, preferred_element_type=f32)
        vs[:, pl.ds(PAD + c * CH, CH)] = jnp.dot(ws[pl.ds(2 * D, D), :], xc, preferred_element_type=f32)

    def attend(c, hh):
        acc = [None] * W
        for d in range(Dh):
            r = d * H + hh * 8
            q = qs[pl.ds(r, 8), pl.ds(c * CH, CH)]
            kf = ks[pl.ds(r, 8), pl.ds(c * CH, CH + PAD)]
            for w in range(W):
                t = q * kf[:, PAD - 2 * w:PAD - 2 * w + CH]
                acc[w] = t if d == 0 else acc[w] + t
        if c == 0:
            lane = jax.lax.broadcasted_iota(jnp.int32, (8, CH), 1)
            acc = [acc[0]] + [jnp.where(lane < 2 * w, -1e9, acc[w]) for w in range(1, W)]
        mx = acc[0]
        for w in range(1, W):
            mx = jnp.maximum(mx, acc[w])
        e = [jnp.exp(a - mx) for a in acc]
        sm = e[0]
        for w in range(1, W):
            sm = sm + e[w]
        pr = [t / sm for t in e]
        for d in range(Dh):
            r = d * H + hh * 8
            vf = vs[pl.ds(r, 8), pl.ds(c * CH, CH + PAD)]
            o = pr[0] * vf[:, PAD:PAD + CH]
            for w in range(1, W):
                o = o + pr[w] * vf[:, PAD - 2 * w:PAD - 2 * w + CH]
            ov[hh, pl.ds(d * 8, 8), :] = o

    def pack(c):
        for d in range(Dh):
            os_[pl.ds(d * H, H), pl.ds(c * CH, CH)] = jnp.concatenate(
                [ov[0, pl.ds(d * 8, 8), :], ov[1, pl.ds(d * 8, 8), :]], axis=0).astype(bf16)

    def mix1(j):
        sl = pl.ds(j * 256, 256)
        u = jnp.dot(xnT[...], w1_v[:, sl], preferred_element_type=f32) + b1_ref[:, sl].astype(f32)
        us[:, sl] = jax.nn.gelu(u, approximate=True).astype(bf16)

    for i in range(8):
        if i < 7:
            c1[i].wait()
            mix1(i)
        attend(i // 2, i % 2)
        if i % 2:
            pack(i // 2)
    for c in c2:
        c.wait()
    for c in range(S // 256):
        sl = pl.ds(c * 256, 256)
        t = jnp.dot(us[...], w2_v[:, sl], preferred_element_type=f32) + b2_ref[:, sl].astype(f32)
        t = t + jnp.dot(woT[...], os_[:, sl], preferred_element_type=f32)
        o_ref[:, sl] = (t + x_ref[:, sl].astype(f32)).astype(bf16)


@jax.jit
def pallas_parallel_sum__sliding_local_dilated__mixer_token_mlp__prompt_kernel(
    A_x, A_wqkv, A_wo, B_x, B_w1, B_b1, B_w2, B_b2):
    x = A_x.transpose(0, 2, 1)
    vm = pl.BlockSpec(memory_space=pltpu.VMEM)
    anys = pl.BlockSpec(memory_space=pl.ANY)
    out = pl.pallas_call(
        _kernel,
        out_shape=jax.ShapeDtypeStruct((1, D, S), bf16),
        grid=(),
        in_specs=[vm, vm, vm, anys, pl.BlockSpec((1, F), lambda: (0, 0)), anys,
                  vm],
        out_specs=pl.BlockSpec((1, D, S), lambda: (0, 0, 0)),
        scratch_shapes=[
            pltpu.VMEM((S, F), bf16), pltpu.VMEM((F, S), bf16),
            pltpu.SemaphoreType.DMA((2, 8)),
            pltpu.VMEM((D, S), bf16), pltpu.VMEM((4, 3 * D, 128), f32),
            pltpu.VMEM((3 * D, D), bf16), pltpu.VMEM((D, D), bf16),
            pltpu.VMEM((D, S), f32), pltpu.VMEM((D, PAD + S), f32), pltpu.VMEM((D, PAD + S), f32),
            pltpu.VMEM((D, S), bf16), pltpu.VMEM((D, F), bf16), pltpu.VMEM((D, D), bf16), pltpu.VMEM((2, Dh * 8, CH), f32),
        ],
        compiler_params=pltpu.CompilerParams(vmem_limit_bytes=112 * 1024 * 1024),
    )(x, A_wqkv, A_wo, B_w1, B_b1.reshape(1, F), B_w2, B_b2.reshape(1, S))
    return out.transpose(0, 2, 1)
```

```python
import jax
import jax.numpy as jnp
import jax.experimental.pallas as pl
import jax.experimental.pallas.tpu as pltpu

S, D, F, H, Dh, W = 2048, 448, 1792, 16, 28, 8
CH = 512
NCH = S // CH
PAD = 128
FC = 256
SC = 256
f32, bf16, i32 = jnp.float32, jnp.bfloat16, jnp.int32


def _unpack(p):
    lo = pltpu.bitcast(jax.lax.shift_left(p, 16), f32)
    hi = pltpu.bitcast(jax.lax.bitwise_and(p, -65536), f32)
    return lo, hi


def _kernel(x_hbm, wqkv_hbm, wo_hbm, w1_hbm, b1_ref, w2_hbm, b2_ref, o_hbm,
            x_v, wqkv_v, wo_v, w1_v, w2_v, o_v, sem_x, sem_w, sem_o,
            wT, ws, woT, xnT, qs, kp, vp, ps, os_, us, y_v):
    def xcopy(c):
        return pltpu.make_async_copy(x_hbm.at[0, :, pl.ds(c * CH, CH)], x_v.at[:, pl.ds(c * CH, CH)], sem_x.at[c])
    cp_wqkv = pltpu.make_async_copy(wqkv_hbm, wqkv_v, sem_w.at[0])
    cp_wo = pltpu.make_async_copy(wo_hbm, wo_v, sem_w.at[1])
    cp_w1 = pltpu.make_async_copy(w1_hbm, w1_v, sem_w.at[2])
    cp_w2 = pltpu.make_async_copy(w2_hbm, w2_v, sem_w.at[3])

    def ocopy(c):
        return pltpu.make_async_copy(o_v.at[:, pl.ds(c * SC, SC)], o_hbm.at[0, :, pl.ds(c * SC, SC)], sem_o.at[c])

    xcopy(0).start()
    cp_wqkv.start()
    for c in range(1, NCH):
        xcopy(c).start()
    cp_wo.start()
    cp_w1.start()

    kp[:, pl.ds(0, PAD)] = jnp.zeros((D // 2, PAD), i32)
    vp[:, pl.ds(0, PAD)] = jnp.zeros((D // 2, PAD), i32)

    def layernorm(c):
        xf = x_v[:, pl.ds(c * CH, CH)].astype(f32)
        m = jnp.mean(xf, axis=0, keepdims=True)
        xc = xf - m
        v = jnp.mean(xc * xc, axis=0, keepdims=True)
        r = 1.0 / jnp.sqrt(v + 1e-5)
        xnT[:, pl.ds(c * CH, CH)] = (xc * r).astype(bf16)

    def stage_T(wf, ncol_tiles, nrows):
        wp = jnp.concatenate([wf, jnp.zeros((64, wf.shape[1]), f32)], axis=0)
        wt = wp.T[:nrows, :]
        for j in range(4):
            wT[j, pl.ds(0, nrows), :] = wt[:, j * 128:(j + 1) * 128]

    def gather(r0, n, stride):
        return jnp.concatenate([wT[j, pl.ds(r0, n, stride=stride), :] for j in range(4)], axis=1)[:, :D]

    scale = Dh ** -0.5

    def prep_qkv():
        wf = wqkv_v[...].astype(f32)
        wf = jnp.concatenate([wf, jnp.zeros((D, 64), f32)], axis=1)
        stage_T(wf, 11, 3 * D)
        for d in range(Dh):
            blk = jnp.concatenate([gather(d, 8, 2 * Dh), gather(Dh + d, 8, 2 * Dh)], axis=0) * scale
            ws[pl.ds(d * H, H), :] = blk.astype(bf16)
        for part in (1, 2):
            for d in range(Dh):
                ws[pl.ds(part * D + d * H, H), :] = gather(part * D + d, H, Dh).astype(bf16)

    def prep_wo():
        wof = jnp.concatenate([wo_v[...].astype(f32), jnp.zeros((D, 64), f32)], axis=1)
        for j in range(4):
            wT[j, pl.ds(0, D), :] = wof[:, j * 128:(j + 1) * 128]
        rows = []
        for d in range(Dh):
            rows.append(gather(d, 8, 2 * Dh))
            rows.append(gather(Dh + d, 8, 2 * Dh))
        wq = jnp.concatenate(rows + [jnp.zeros((64, D), f32)], axis=0)
        wq = jnp.concatenate([wq, jnp.zeros((512, 64), f32)], axis=1)
        woT[...] = wq.T[:D, :D].astype(bf16)

    def qkv(c):
        xc = xnT[:, pl.ds(c * CH, CH)]
        qs[:, pl.ds(c * CH, CH)] = jnp.dot(ws[pl.ds(0, D), :], xc, preferred_element_type=f32)
        k = jnp.dot(ws[pl.ds(D, D), :], xc, preferred_element_type=f32)
        kp[:, pl.ds(PAD + c * CH, CH)] = pltpu.bitcast(k.astype(bf16), i32)
        v = jnp.dot(ws[pl.ds(2 * D, D), :], xc, preferred_element_type=f32)
        vp[:, pl.ds(PAD + c * CH, CH)] = pltpu.bitcast(v.astype(bf16), i32)

    def shifted(ref, d, c, w):
        if w == 0:
            return ref[pl.ds(d * 8, 8), pl.ds(PAD + c * CH, CH)]
        full = ref[pl.ds(d * 8, 8), pl.ds(c * CH, CH + PAD)]
        return pltpu.roll(full, 2 * w, 1)[:, PAD:]

    def qk(c, ws_):
        acc = {}
        for d in range(Dh):
            qlo = qs[pl.ds(d * H, 8), pl.ds(c * CH, CH)]
            qhi = qs[pl.ds(d * H + 8, 8), pl.ds(c * CH, CH)]
            for w in ws_:
                lo, hi = _unpack(shifted(kp, d, c, w))
                tlo, thi = qlo * lo, qhi * hi
                acc[w] = (tlo, thi) if d == 0 else (acc[w][0] + tlo, acc[w][1] + thi)
        for w in ws_:
            alo, ahi = acc[w]
            if w > 0 and c == 0:
                lane = jax.lax.broadcasted_iota(i32, (8, CH), 1)
                alo = jnp.where(lane < 2 * w, -1e9, alo)
                ahi = jnp.where(lane < 2 * w, -1e9, ahi)
            ps[w, pl.ds(0, 8), :] = alo
            ps[w, pl.ds(8, 8), :] = ahi

    def softmax(c):
        lg = [ps[w] for w in range(W)]
        mx = lg[0]
        for w in range(1, W):
            mx = jnp.maximum(mx, lg[w])
        e = [jnp.exp(a - mx) for a in lg]
        sm = e[0]
        for w in range(1, W):
            sm = sm + e[w]
        r = 1.0 / sm
        for w in range(W):
            ps[w] = e[w] * r

    def pv(c, ds_):
        for d in ds_:
            olo = ohi = None
            for w in range(W):
                lo, hi = _unpack(shifted(vp, d, c, w))
                tlo = ps[w, pl.ds(0, 8), :] * lo
                thi = ps[w, pl.ds(8, 8), :] * hi
                olo, ohi = (tlo, thi) if w == 0 else (olo + tlo, ohi + thi)
            os_[pl.ds(d * H, H), pl.ds(c * CH, CH)] = jnp.concatenate([olo, ohi], axis=0).astype(bf16)

    def att_pieces(c):
        yield lambda: qk(c, range(0, 4))
        yield lambda: qk(c, range(4, 8))

        def p2():
            softmax(c)
            pv(c, range(0, Dh // 2))
        yield p2
        yield lambda: pv(c, range(Dh // 2, Dh))

    def mix1(j):
        sl = pl.ds(j * FC, FC)
        u = jnp.dot(xnT[...], w1_v[:, sl], preferred_element_type=f32) + b1_ref[:, sl].astype(f32)
        us[:, sl] = jax.nn.gelu(u, approximate=True).astype(bf16)

    def mix2(c):
        sl = pl.ds(c * SC, SC)
        y_v[:, sl] = jnp.dot(us[...], w2_v[:, sl], preferred_element_type=f32) + b2_ref[:, sl].astype(f32)

    def final(c):
        sl = pl.ds(c * SC, SC)
        t = jnp.dot(woT[...], os_[:, sl], preferred_element_type=f32)
        o_v[:, sl] = (t + y_v[:, sl] + x_v[:, sl].astype(f32)).astype(bf16)
        ocopy(c).start()

    xcopy(0).wait()
    cp_wqkv.wait()
    layernorm(0)
    prep_qkv()
    for c in range(1, NCH):
        xcopy(c).wait()
    cp_wo.wait()
    for c in range(NCH):
        if c + 1 < NCH:
            layernorm(c + 1)
        if c == 0:
            prep_wo()
        qkv(c)
    cp_w1.wait()
    cp_w2.start()
    pieces = [p for c in range(NCH) for p in att_pieces(c)]
    it = iter(pieces)
    for j in range(F // FC):
        mix1(j)
        p = next(it, None)
        if p is not None:
            p()
    cp_w2.wait()
    for c in range(S // SC):
        mix2(c)
        p = next(it, None)
        if p is not None:
            p()
    for p in it:
        p()
    for c in range(S // SC):
        final(c)
    for c in range(S // SC):
        ocopy(c).wait()


@jax.jit
def pallas_parallel_sum__sliding_local_dilated__mixer_token_mlp__prompt_kernel(
        A_x, A_wqkv, A_wo, B_x, B_w1, B_b1, B_w2, B_b2):
    x = A_x.transpose(0, 2, 1)
    vm = pl.BlockSpec(memory_space=pltpu.VMEM)
    anys = pl.BlockSpec(memory_space=pl.ANY)
    out = pl.pallas_call(
        _kernel,
        out_shape=jax.ShapeDtypeStruct((1, D, S), bf16),
        in_specs=[anys, anys, anys, anys, vm, anys, vm],
        out_specs=anys,
        scratch_shapes=[
            pltpu.VMEM((D, S), bf16),
            pltpu.VMEM((D, 3 * D), bf16),
            pltpu.VMEM((D, D), bf16),
            pltpu.VMEM((S, F), bf16),
            pltpu.VMEM((F, S), bf16),
            pltpu.VMEM((D, S), bf16),
            pltpu.SemaphoreType.DMA((NCH,)),
            pltpu.SemaphoreType.DMA((4,)),
            pltpu.SemaphoreType.DMA((S // SC,)),
            pltpu.VMEM((4, 3 * D, 128), f32),
            pltpu.VMEM((3 * D, D), bf16),
            pltpu.VMEM((D, D), bf16),
            pltpu.VMEM((D, S), bf16),
            pltpu.VMEM((D, S), f32),
            pltpu.VMEM((D // 2, PAD + S), i32),
            pltpu.VMEM((D // 2, PAD + S), i32),
            pltpu.VMEM((W, H, CH), f32),
            pltpu.VMEM((D, S), bf16),
            pltpu.VMEM((D, F), bf16),
            pltpu.VMEM((D, S), f32),
        ],
        compiler_params=pltpu.CompilerParams(vmem_limit_bytes=112 * 1024 * 1024),
    )(x, A_wqkv, A_wo, B_w1, B_b1.reshape(1, F), B_w2, B_b2.reshape(1, S))
    return out.transpose(0, 2, 1)
```

```python
import jax
import jax.numpy as jnp
import jax.experimental.pallas as pl
import jax.experimental.pallas.tpu as pltpu

S, D, F, H, Dh, W = 2048, 448, 1792, 16, 28, 8
CH = 512
NCH = S // CH
AC = 128
LNC = 256
PAD = 128
FC = 256
SC = 256
f32, bf16, i32 = jnp.float32, jnp.bfloat16, jnp.int32


def _unpack(p):
    lo = pltpu.bitcast(jax.lax.shift_left(p, 16), f32)
    hi = pltpu.bitcast(jax.lax.bitwise_and(p, -65536), f32)
    return lo, hi


def _pk(v):
    return pltpu.bitcast(v.astype(bf16), i32)


def _up(v):
    return pltpu.bitcast(v, bf16)


def _kernel(x_hbm, wqkv_hbm, wo_hbm, w1_hbm, b1_hbm, w2_hbm, b2_hbm, o_hbm,
            x_v, wqkv_v, wo_v, w1_v, w2_v, o_v, sem,
            wT, ws, woT, xnT, qs, kp, vp, os_, us, y_v, b1_ref, b2_ref):
    def xcopy(c):
        return pltpu.make_async_copy(x_hbm.at[0, :, pl.ds(c * CH, CH)], x_v.at[:, pl.ds(c * CH, CH)], sem.at[1 if c == 0 else 3 if c == 1 else 5])
    wcols = [(0, 512), (512, 384), (896, 448)]
    cp_wqkv = [pltpu.make_async_copy(wqkv_hbm.at[:, pl.ds(a, n)], wqkv_v.at[:, pl.ds(a, n)], sem.at[0 if i == 0 else 2 if i == 1 else 5])
               for i, (a, n) in enumerate(wcols)]
    cp_wo = pltpu.make_async_copy(wo_hbm, wo_v, sem.at[4])
    cp_w1 = pltpu.make_async_copy(w1_hbm, w1_v, sem.at[4])
    cp_b1 = pltpu.make_async_copy(b1_hbm, b1_ref, sem.at[4])
    cp_b2 = pltpu.make_async_copy(b2_hbm, b2_ref, sem.at[4])
    cp_w2 = pltpu.make_async_copy(w2_hbm, w2_v, sem.at[0])

    def ocopy(a, n):
        return pltpu.make_async_copy(o_v.at[:, pl.ds(a, n)], o_hbm.at[0, :, pl.ds(a, n)], sem.at[1])

    cp_wqkv[0].start()
    xcopy(0).start()

    kp[:, pl.ds(0, PAD)] = jnp.zeros((D // 2, PAD), i32)
    vp[:, pl.ds(0, PAD)] = jnp.zeros((D // 2, PAD), i32)

    def layernorm(c):
        for t in range(CH // LNC):
            sl = pl.ds(c * CH + t * LNC, LNC)
            xf = x_v[:, sl].astype(f32)
            m = jnp.mean(xf, axis=0, keepdims=True)
            xc = xf - m
            v = jnp.mean(xc * xc, axis=0, keepdims=True)
            r = 1.0 / jnp.sqrt(v + 1e-5)
            xnT[:, sl] = _pk(xc * r)

    def gather(r0, n, stride):
        return jnp.concatenate([wT[j, pl.ds(r0, n, stride=stride), :] for j in range(4)], axis=1)[:, :D]

    scale = Dh ** -0.5

    def prep_part(part):
        t0 = (part * D) // 128
        t1 = min(11, (part * D + D + 127) // 128)
        for t in range(t0 if part == 0 else (part * D + 127) // 128 if part == 1 else t0, t1):
            width = min(128, 3 * D - t * 128)
            wf = wqkv_v[:, pl.ds(t * 128, width)].astype(f32)
            if width < 128:
                wf = jnp.concatenate([wf, jnp.zeros((D, 128 - width), f32)], axis=1)
            wp = jnp.concatenate([wf, jnp.zeros((64, 128), f32)], axis=0)
            wt = wp.T[:width, :]
            for j in range(4):
                wT[j, pl.ds(t * 128, width), :] = wt[:, j * 128:(j + 1) * 128]
        for d in range(Dh):
            if part == 0:
                blk = jnp.concatenate([gather(d, 8, 2 * Dh), gather(Dh + d, 8, 2 * Dh)], axis=0) * scale
            else:
                blk = gather(part * D + d, H, Dh)
            ws[pl.ds((part * D + d * H) // 2, 8), :] = _pk(blk)

    def prep_wo():
        wof = jnp.concatenate([wo_v[...].astype(f32), jnp.zeros((D, 64), f32)], axis=1)
        for j in range(4):
            wT[j, pl.ds(0, D), :] = wof[:, j * 128:(j + 1) * 128]
        rows = []
        for d in range(Dh):
            rows.append(gather(d, 8, 2 * Dh))
            rows.append(gather(Dh + d, 8, 2 * Dh))
        wq = jnp.concatenate(rows + [jnp.zeros((64, D), f32)], axis=0)
        wq = jnp.concatenate([wq, jnp.zeros((512, 64), f32)], axis=1)
        woT[...] = _pk(wq.T[:D, :D])

    def mm_q(c, off=0, n=CH):
        qs[:, pl.ds(c * CH + off, n)] = jnp.dot(_up(ws[pl.ds((0) // 2, D // 2), :]), _up(xnT[:, pl.ds(c * CH + off, n)]), preferred_element_type=f32)

    def mm_k(c, off=0, n=CH):
        k = jnp.dot(_up(ws[pl.ds((D) // 2, D // 2), :]), _up(xnT[:, pl.ds(c * CH + off, n)]), preferred_element_type=f32)
        kp[:, pl.ds(PAD + c * CH + off, n)] = pltpu.bitcast(k.astype(bf16), i32)

    def mm_v(c, off=0, n=CH):
        v = jnp.dot(_up(ws[pl.ds((2 * D) // 2, D // 2), :]), _up(xnT[:, pl.ds(c * CH + off, n)]), preferred_element_type=f32)
        vp[:, pl.ds(PAD + c * CH + off, n)] = pltpu.bitcast(v.astype(bf16), i32)

    def shifted(ref, d, c, w):
        if w == 0:
            return ref[pl.ds(d * 8, 8), pl.ds(PAD + c * AC, AC)]
        full = ref[pl.ds(d * 8, 8), pl.ds(c * AC, AC + PAD)]
        return pltpu.roll(full, 2 * w, 1)[:, PAD:]

    def attend(c):
        acc = [None] * W
        for d in range(Dh):
            qlo = qs[pl.ds(d * H, 8), pl.ds(c * AC, AC)]
            qhi = qs[pl.ds(d * H + 8, 8), pl.ds(c * AC, AC)]
            for w in range(W):
                lo, hi = _unpack(shifted(kp, d, c, w))
                tlo, thi = qlo * lo, qhi * hi
                acc[w] = (tlo, thi) if d == 0 else (acc[w][0] + tlo, acc[w][1] + thi)
        p = []
        for half in range(2):
            lg = [acc[w][half] for w in range(W)]
            if c * AC < 2 * W:
                lane = c * AC + jax.lax.broadcasted_iota(i32, (8, AC), 1)
                lg = [lg[0]] + [jnp.where(lane < 2 * w, -1e9, lg[w]) for w in range(1, W)]
            mx = lg[0]
            for w in range(1, W):
                mx = jnp.maximum(mx, lg[w])
            e = [jnp.exp(a - mx) for a in lg]
            sm = e[0]
            for w in range(1, W):
                sm = sm + e[w]
            r = 1.0 / sm
            p.append([t * r for t in e])
        for d in range(Dh):
            olo = ohi = None
            for w in range(W):
                lo, hi = _unpack(shifted(vp, d, c, w))
                tlo, thi = p[0][w] * lo, p[1][w] * hi
                olo, ohi = (tlo, thi) if w == 0 else (olo + tlo, ohi + thi)
            os_[pl.ds(d * 8, 8), pl.ds(c * AC, AC)] = _pk(jnp.concatenate([olo, ohi], axis=0))

    def mix1(j):
        sl = pl.ds(j * FC, FC)
        u = jnp.dot(_up(xnT[...]), w1_v[:, sl], preferred_element_type=f32) + b1_ref[sl].astype(f32).reshape(1, FC)
        us[:, sl] = _pk(jax.nn.gelu(u, approximate=True))

    def mix2(c):
        sl = pl.ds(c * SC, SC)
        y_v[:, sl] = jnp.dot(_up(us[...]), w2_v[:, sl], preferred_element_type=f32) + b2_ref[sl].astype(f32).reshape(1, SC)

    def final(a, n):
        sl = pl.ds(a, n)
        t = jnp.dot(_up(woT[...]), _up(os_[:, sl]), preferred_element_type=f32)
        o_v[:, sl] = (t + y_v[:, sl] + x_v[:, sl].astype(f32)).astype(bf16)
        ocopy(a, n).start()

    cp_wqkv[0].wait()
    cp_wqkv[1].start()
    xcopy(1).start()
    prep_part(0)
    xcopy(0).wait()
    cp_wqkv[2].start()
    xcopy(2).start()
    xcopy(3).start()
    layernorm(0)
    mm_q(0, 0, 384)
    cp_wqkv[1].wait()
    xcopy(1).wait()
    cp_w1.start()
    cp_wo.start()
    cp_b1.start()
    cp_b2.start()
    mm_q(0, 384, CH - 384)
    layernorm(1)
    mm_q(1)
    prep_part(1)
    mm_k(0)
    mm_k(1, 0, 256)
    cp_wqkv[2].wait()
    xcopy(2).wait()
    xcopy(3).wait()
    mm_k(1, 256, 256)
    prep_part(2)
    layernorm(2)
    layernorm(3)
    mm_v(0)
    mm_v(1)
    todo = list(range(S // AC))

    def att(n):
        for _ in range(n):
            if todo:
                attend(todo.pop(0))

    for c in range(2, NCH):
        mm_q(c)
        mm_k(c)
        mm_v(c)
    cp_wo.wait()
    cp_b1.wait()
    cp_b2.wait()
    cp_w1.wait()
    cp_w2.start()
    prep_wo()
    for j in range(F // FC):
        mix1(j)
        att(1)
    cp_w2.wait()
    for c in range(S // SC):
        mix2(c)
        att(2)
    att(100)
    fchunks = [(c * 256, 256) for c in range(7)] + [(1792, 128), (1920, 128)]
    for a, n in fchunks:
        final(a, n)
    for a, n in fchunks:
        ocopy(a, n).wait()


@jax.jit
def pallas_parallel_sum__sliding_local_dilated__mixer_token_mlp__prompt_kernel(
        A_x, A_wqkv, A_wo, B_x, B_w1, B_b1, B_w2, B_b2):
    x = A_x.transpose(0, 2, 1)
    anys = pl.BlockSpec(memory_space=pl.ANY)
    out = pl.pallas_call(
        _kernel,
        out_shape=jax.ShapeDtypeStruct((1, D, S), bf16),
        in_specs=[anys] * 7,
        out_specs=anys,
        scratch_shapes=[
            pltpu.VMEM((D, S), bf16),
            pltpu.VMEM((D, 3 * D), bf16),
            pltpu.VMEM((D, D), bf16),
            pltpu.VMEM((S, F), bf16),
            pltpu.VMEM((F, S), bf16),
            pltpu.VMEM((D, S), bf16),
            pltpu.SemaphoreType.DMA((6,)),
            pltpu.VMEM((4, 3 * D, 128), f32),
            pltpu.VMEM((3 * D // 2, D), i32),
            pltpu.VMEM((D // 2, D), i32),
            pltpu.VMEM((D // 2, S), i32),
            pltpu.VMEM((D, S), f32),
            pltpu.VMEM((D // 2, PAD + S), i32),
            pltpu.VMEM((D // 2, PAD + S), i32),
            pltpu.VMEM((D // 2, S), i32),
            pltpu.VMEM((D // 2, F), i32),
            pltpu.VMEM((D, S), f32),
            pltpu.VMEM((F,), bf16), pltpu.VMEM((S,), bf16),
        ],
        compiler_params=pltpu.CompilerParams(vmem_limit_bytes=112 * 1024 * 1024, flags={"XLA_TPU_EVENLY_DISTRIBUTE_CRITICAL_NODES": True}),
    )(x, A_wqkv, A_wo, B_w1, B_b1, B_w2, B_b2)
    return out.transpose(0, 2, 1)
```

```python
import jax
import jax.numpy as jnp
import jax.experimental.pallas as pl
import jax.experimental.pallas.tpu as pltpu

S, D, F, H, Dh, W = 2048, 448, 1792, 16, 28, 8
CH = 512
NCH = S // CH
AC = 128
LNC = 256
PAD = 128
FC = 256
SC = 256
f32, bf16, i32 = jnp.float32, jnp.bfloat16, jnp.int32


def _unpack(p):
    lo = pltpu.bitcast(jax.lax.shift_left(p, 16), f32)
    hi = pltpu.bitcast(jax.lax.bitwise_and(p, -65536), f32)
    return lo, hi


def _pk(v):
    return pltpu.bitcast(v.astype(bf16), i32)


def _up(v):
    return pltpu.bitcast(v, bf16)


def _kernel(x_hbm, wqkv_hbm, wo_hbm, w1_hbm, b1_hbm, w2_hbm, b2_hbm, o_hbm,
            x_v, wqkv_v, wo_v, w1_v, w2_v, o_v, sem,
            wT, ws, woT, xnT, qs, kp, vp, os_, us, y_v, b1_ref, b2_ref):
    def xcopy(c):
        return pltpu.make_async_copy(x_hbm.at[0, :, pl.ds(c * CH, CH)], x_v.at[:, pl.ds(c * CH, CH)], sem.at[1 if c == 0 else 3 if c == 1 else 5])
    wcols = [(0, 512), (512, 384), (896, 448)]
    cp_wqkv = [pltpu.make_async_copy(wqkv_hbm.at[:, pl.ds(a, n)], wqkv_v.at[:, pl.ds(a, n)], sem.at[0 if i == 0 else 2 if i == 1 else 5])
               for i, (a, n) in enumerate(wcols)]
    cp_wo = pltpu.make_async_copy(wo_hbm, wo_v, sem.at[4])
    cp_w1 = pltpu.make_async_copy(w1_hbm, w1_v, sem.at[4])
    cp_b1 = pltpu.make_async_copy(b1_hbm, b1_ref, sem.at[4])
    cp_b2 = pltpu.make_async_copy(b2_hbm, b2_ref, sem.at[4])
    cp_w2 = pltpu.make_async_copy(w2_hbm, w2_v.at[:, pl.ds(0, S)], sem.at[0])

    def ocopy(a, n, r0=0, nr=D):
        rs, sl = pl.ds(r0, nr), pl.ds(a, n)
        return pltpu.make_async_copy(o_v.at[rs, sl], o_hbm.at[0, rs, sl], sem.at[1])

    cp_wqkv[0].start()
    xcopy(0).start()

    kp[:, pl.ds(0, PAD)] = jnp.zeros((D // 2, PAD), i32)
    vp[:, pl.ds(0, PAD)] = jnp.zeros((D // 2, PAD), i32)

    def layernorm(c):
        for t in range(CH // LNC):
            sl = pl.ds(c * CH + t * LNC, LNC)
            xf = x_v[:, sl].astype(f32)
            m = jnp.mean(xf, axis=0, keepdims=True)
            xc = xf - m
            v = jnp.mean(xc * xc, axis=0, keepdims=True)
            r = 1.0 / jnp.sqrt(v + 1e-5)
            xnT[:, sl] = _pk(xc * r)

    def gather(r0, n, stride):
        return jnp.concatenate([wT[j, pl.ds(r0, n, stride=stride), :] for j in range(4)], axis=1)[:, :D]

    scale = Dh ** -0.5

    def prep_part(part):
        t0 = (part * D) // 128
        t1 = min(11, (part * D + D + 127) // 128)
        for t in range(t0 if part == 0 else (part * D + 127) // 128 if part == 1 else t0, t1):
            width = min(128, 3 * D - t * 128)
            wf = wqkv_v[:, pl.ds(t * 128, width)].astype(f32)
            if width < 128:
                wf = jnp.concatenate([wf, jnp.zeros((D, 128 - width), f32)], axis=1)
            wp = jnp.concatenate([wf, jnp.zeros((64, 128), f32)], axis=0)
            wt = wp.T[:width, :]
            for j in range(4):
                wT[j, pl.ds(t * 128, width), :] = wt[:, j * 128:(j + 1) * 128]
        for d in range(Dh):
            if part == 0:
                blk = jnp.concatenate([gather(d, 8, 2 * Dh), gather(Dh + d, 8, 2 * Dh)], axis=0) * scale
            else:
                blk = gather(part * D + d, H, Dh)
            ws[pl.ds((part * D + d * H) // 2, 8), :] = _pk(blk)

    def prep_wo():
        wof = jnp.concatenate([wo_v[...].astype(f32), jnp.zeros((D, 64), f32)], axis=1)
        for j in range(4):
            wT[j, pl.ds(0, D), :] = wof[:, j * 128:(j + 1) * 128]
        rows = []
        for d in range(Dh):
            rows.append(gather(d, 8, 2 * Dh))
            rows.append(gather(Dh + d, 8, 2 * Dh))
        wq = jnp.concatenate(rows + [jnp.zeros((64, D), f32)], axis=0)
        wq = jnp.concatenate([wq, jnp.zeros((512, 64), f32)], axis=1)
        woT[...] = _pk(wq.T[:D, :D])

    def mm_q(c, off=0, n=CH):
        qs[:, pl.ds(c * CH + off, n)] = jnp.dot(_up(ws[pl.ds((0) // 2, D // 2), :]), _up(xnT[:, pl.ds(c * CH + off, n)]), preferred_element_type=f32)

    def mm_k(c, off=0, n=CH):
        k = jnp.dot(_up(ws[pl.ds((D) // 2, D // 2), :]), _up(xnT[:, pl.ds(c * CH + off, n)]), preferred_element_type=f32)
        kp[:, pl.ds(PAD + c * CH + off, n)] = pltpu.bitcast(k.astype(bf16), i32)

    def mm_v(c, off=0, n=CH):
        v = jnp.dot(_up(ws[pl.ds((2 * D) // 2, D // 2), :]), _up(xnT[:, pl.ds(c * CH + off, n)]), preferred_element_type=f32)
        vp[:, pl.ds(PAD + c * CH + off, n)] = pltpu.bitcast(v.astype(bf16), i32)

    def shifted(ref, d, c, w):
        if w == 0:
            return ref[pl.ds(d * 8, 8), pl.ds(PAD + c * AC, AC)]
        full = ref[pl.ds(d * 8, 8), pl.ds(c * AC, AC + PAD)]
        return pltpu.roll(full, 2 * w, 1)[:, PAD:]

    def attend(c):
        acc = [None] * W
        for d in range(Dh):
            qlo = qs[pl.ds(d * H, 8), pl.ds(c * AC, AC)]
            qhi = qs[pl.ds(d * H + 8, 8), pl.ds(c * AC, AC)]
            for w in range(W):
                lo, hi = _unpack(shifted(kp, d, c, w))
                tlo, thi = qlo * lo, qhi * hi
                acc[w] = (tlo, thi) if d == 0 else (acc[w][0] + tlo, acc[w][1] + thi)
        p = []
        for half in range(2):
            lg = [acc[w][half] for w in range(W)]
            if c * AC < 2 * W:
                lane = c * AC + jax.lax.broadcasted_iota(i32, (8, AC), 1)
                lg = [lg[0]] + [jnp.where(lane < 2 * w, -1e9, lg[w]) for w in range(1, W)]
            mx = lg[0]
            for w in range(1, W):
                mx = jnp.maximum(mx, lg[w])
            e = [jnp.exp(a - mx) for a in lg]
            sm = e[0]
            for w in range(1, W):
                sm = sm + e[w]
            r = 1.0 / sm
            p.append([t * r for t in e])
        for d in range(Dh):
            olo = ohi = None
            for w in range(W):
                lo, hi = _unpack(shifted(vp, d, c, w))
                tlo, thi = p[0][w] * lo, p[1][w] * hi
                olo, ohi = (tlo, thi) if w == 0 else (olo + tlo, ohi + thi)
            os_[pl.ds(d * 8, 8), pl.ds(c * AC, AC)] = _pk(jnp.concatenate([olo, ohi], axis=0))

    def mix1(j):
        sl = pl.ds(j * FC, FC)
        u = jnp.dot(_up(xnT[...]), w1_v[:, sl], preferred_element_type=f32) + b1_ref[sl].astype(f32).reshape(1, FC)
        us[:, sl] = _pk(jax.nn.gelu(u, approximate=True))

    def mix2(c):
        sl = pl.ds(c * SC, SC)
        y_v[:, sl] = jnp.dot(_up(us[...]), w2_v[:, sl], preferred_element_type=f32) + b2_ref[sl].astype(f32).reshape(1, SC)

    def final(a, n, r0=0, nr=D):
        sl, rs = pl.ds(a, n), pl.ds(r0, nr)
        t = jnp.dot(_up(woT[pl.ds(r0 // 2, nr // 2), :]), _up(os_[:, sl]), preferred_element_type=f32)
        o_v[rs, sl] = (t + y_v[rs, sl] + x_v[rs, sl].astype(f32)).astype(bf16)
        ocopy(a, n, r0, nr).start()

    cp_wqkv[0].wait()
    cp_wqkv[1].start()
    xcopy(1).start()
    prep_part(0)
    xcopy(0).wait()
    cp_wqkv[2].start()
    xcopy(2).start()
    xcopy(3).start()
    layernorm(0)
    mm_q(0, 0, 384)
    cp_wqkv[1].wait()
    xcopy(1).wait()
    cp_w1.start()
    cp_wo.start()
    cp_b1.start()
    cp_b2.start()
    mm_q(0, 384, CH - 384)
    layernorm(1)
    mm_q(1)
    prep_part(1)
    mm_k(0)
    mm_k(1, 0, 256)
    cp_wqkv[2].wait()
    xcopy(2).wait()
    xcopy(3).wait()
    mm_k(1, 256, 256)
    prep_part(2)
    layernorm(2)
    layernorm(3)
    mm_v(0)
    mm_v(1)
    todo = list(range(S // AC))

    def att(n):
        for _ in range(n):
            if todo:
                attend(todo.pop(0))

    for c in range(2, NCH):
        mm_q(c)
        mm_k(c)
        mm_v(c)
    cp_wo.wait()
    cp_b1.wait()
    cp_b2.wait()
    cp_w1.wait()
    cp_w2.start()
    for j in range(F // FC):
        mix1(j)
        att(1)
    prep_wo()
    cp_w2.wait()
    for c in range(S // SC):
        mix2(c)
        att(2)
    att(100)
    fchunks = [(c * 256, 256) for c in range(7)] + [(1792, 128), (1920, 128, 0, 224), (1920, 128, 224, 224)]
    for fc in fchunks:
        final(*fc)
    for fc in fchunks:
        ocopy(*fc).wait()


@jax.jit
def pallas_parallel_sum__sliding_local_dilated__mixer_token_mlp__prompt_kernel(
        A_x, A_wqkv, A_wo, B_x, B_w1, B_b1, B_w2, B_b2):
    x = A_x.transpose(0, 2, 1)
    anys = pl.BlockSpec(memory_space=pl.ANY)
    out = pl.pallas_call(
        _kernel,
        out_shape=jax.ShapeDtypeStruct((1, D, S), bf16),
        in_specs=[anys] * 7,
        out_specs=anys,
        scratch_shapes=[
            pltpu.VMEM((D, S), bf16),
            pltpu.VMEM((D, 3 * D), bf16),
            pltpu.VMEM((D, D), bf16),
            pltpu.VMEM((S, F), bf16),
            pltpu.VMEM((F, S + 128), bf16),
            pltpu.VMEM((D, S), bf16),
            pltpu.SemaphoreType.DMA((6,)),
            pltpu.VMEM((4, 3 * D, 128), f32),
            pltpu.VMEM((3 * D // 2, D), i32),
            pltpu.VMEM((D // 2, D), i32),
            pltpu.VMEM((D // 2, S), i32),
            pltpu.VMEM((D, S), f32),
            pltpu.VMEM((D // 2, PAD + S), i32),
            pltpu.VMEM((D // 2, PAD + S), i32),
            pltpu.VMEM((D // 2, S), i32),
            pltpu.VMEM((D // 2, F), i32),
            pltpu.VMEM((D, S), f32),
            pltpu.VMEM((F,), bf16), pltpu.VMEM((S,), bf16),
        ],
        compiler_params=pltpu.CompilerParams(vmem_limit_bytes=112 * 1024 * 1024, flags={"XLA_TPU_EVENLY_DISTRIBUTE_CRITICAL_NODES": True}),
    )(x, A_wqkv, A_wo, B_w1, B_b1, B_w2, B_b2)
    return out.transpose(0, 2, 1)
```
